```python
import os as _os
_os.environ.setdefault("JAX_PLATFORMS", "cpu")
import jax
import jax.numpy as jnp

def _softmax(x, axis=-1):
    return jax.nn.softmax(x, axis=axis)
def _gelu(x):
    return jax.nn.gelu(x, approximate=True)
def _silu(x):
    return jax.nn.silu(x)
def _sigmoid(x):
    return jax.nn.sigmoid(x)
def _layernorm(x, axis=-1, eps=1e-5):
    m = jnp.mean(x, axis=axis, keepdims=True)
    v = jnp.var(x, axis=axis, keepdims=True)
    return (x - m) / jnp.sqrt(v + eps)
def _scatter_add(tgt, idx, src, axis=0):
    return tgt.at[idx].add(src)
def _segment_sum(src, seg, n):
    return jax.ops.segment_sum(src, seg, n)
class _Rng:
    def __init__(self, key):
        self._k = key
    def _next(self):
        self._k, sub = jax.random.split(self._k)
        return sub
    def normal(self, shape):
        return jax.random.normal(self._next(), shape, dtype=jnp.bfloat16)
    def randint(self, lo, hi, shape):
        return jax.random.randint(self._next(), shape, lo, hi, dtype=jnp.int32)
    def uniform(self, shape, lo=0.0, hi=1.0):
        return jax.random.uniform(self._next(), shape, jnp.bfloat16, lo, hi)
    def permutation(self, n):
        return jax.random.permutation(self._next(), n)


kernel_name = 'standalone__channel_attn_cbam__vision'

def setup_inputs():
    _rng = _Rng(jax.random.key(int.from_bytes(__import__("os").urandom(4), "little")))
    _w = (lambda a: (lambda t: t.astype(jnp.bfloat16) if jnp.issubdtype(t.dtype, jnp.floating) else t)(jnp.asarray(a)))
    H = W = 224
    C = 192
    r = max(C // 4, 1)
    return {
        "x": _w((lambda *s: _rng.normal(s) * 0.2)(1, H, W, C) + (lambda *s: _rng.normal(s) * 0.2)(1, 1, 1, C) * 2.0),
        "w1": _w((lambda *s: _rng.normal(s) * 0.2)(C, r)),
        "w2": _w((lambda *s: _rng.normal(s) * 0.2)(r, C)),
    }

def reference(x, w1, w2):
    B, H, W, C = x.shape
    xf = x.reshape(B, H * W, C)
    gap = jnp.mean(xf, 1)
    gmp = jnp.amax(xf, 1)
    h_a = gap @ w1
    h_a = h_a * (lambda x, dt: x.astype(dt))(h_a > 0, h_a.dtype)
    h_m = gmp @ w1
    h_m = h_m * (lambda x, dt: x.astype(dt))(h_m > 0, h_m.dtype)
    scale = _sigmoid(h_a @ w2 + h_m @ w2)
    return x * scale[:, None, None, :]
```

```python
import math

import jax
import jax.numpy as jnp
from jax import lax
import jax.experimental.pallas as pl
import jax.experimental.pallas.tpu as pltpu

F32, BF16 = jnp.float32, jnp.bfloat16
LANES = 128

READ_CHUNKS = (124, 60, 24, 9, 4, 3)
SLAB = 1024
HEAD, PIECE = (8, 40), 48


def _make_kernel(H, C, W):
    n_slab = H * C // SLAB
    period = C // math.gcd(SLAB % C, C)
    n_piece = (SLAB - sum(HEAD)) // PIECE
    tail = SLAB - sum(HEAD) - n_piece * PIECE
    n_read = len(READ_CHUNKS)
    row0 = [sum(READ_CHUNKS[:i]) for i in range(n_read)]

    def kernel(x_hbm, w1t_hbm, w2_hbm, o_hbm, xbuf, obuf, w1v, w2v, w1f, w2f,
               acc_s, acc_m, scale, wsem):

        def body(rsem, psem):
            reads = [
                pltpu.make_async_copy(x_hbm.at[pl.ds(h0 * C, n * C)],
                                      xbuf.at[pl.ds(h0 * C, n * C)], rsem.at[i])
                for i, (h0, n) in enumerate(zip(row0, READ_CHUNKS))
            ]
            w1_copy = pltpu.make_async_copy(w1t_hbm, w1v, psem)
            w2_copy = pltpu.make_async_copy(w2_hbm, w2v, psem)
            w1_copy.start()
            w2_copy.start()
            for c in reads:
                c.start(priority=1)
            acc_s[...] = jnp.zeros((C, W), F32)
            acc_m[...] = jnp.full((C, W), -jnp.inf, F32)
            w1_copy.wait()
            w2_copy.wait()
            w1f[...] = w1v[...].astype(F32).T
            w2f[...] = w2v[...].astype(F32).T

            for i in range(n_read - 1):
                reads[i].wait()
                n = READ_CHUNKS[i]
                u = 4 if (n % 4 == 0 and n > 9) else n

                def channels(cg, carry, h0=row0[i], n=n, u=u):
                    c0 = pl.multiple_of(cg * 16, 16)

                    def step(b, sm):
                        s, m = sm
                        for q in range(u):
                            r = pl.multiple_of((h0 + b * u + q) * C + c0, 16)
                            v = xbuf[pl.ds(r, 16), :].astype(F32)
                            s, m = s + v, jnp.maximum(m, v)
                        return s, m

                    sm = (acc_s[pl.ds(c0, 16), :], acc_m[pl.ds(c0, 16), :])
                    s, m = step(0, sm) if n == u else lax.fori_loop(0, n // u, step, sm)
                    acc_s[pl.ds(c0, 16), :] = s
                    acc_m[pl.ds(c0, 16), :] = m
                    return carry

                lax.fori_loop(0, C // 16, channels, 0)

            def start_write(j0, n):
                pltpu.make_async_copy(obuf.at[:, pl.ds(j0, n)],
                                      o_hbm.at[:, pl.ds(j0, n)], wsem).start()

            def apply(j, scales):
                for p in range(period):
                    sv = jnp.concatenate([scales[p], scales[p][:, :W - LANES]], axis=1)
                    for n in range(p, n_slab, period):
                        v = xbuf[pl.ds(pl.multiple_of(n * SLAB + j, 8), 8), :].astype(F32)
                        obuf[n, pl.ds(pl.multiple_of(j, 8), 8), :] = (v * sv).astype(BF16)

            reads[-1].wait()
            ha = hm = None
            for c0 in range(0, C, 8):
                s, m = acc_s[c0:c0 + 8, :], acc_m[c0:c0 + 8, :]
                for h in range(row0[-1], H):
                    v = xbuf[h * C + c0:h * C + c0 + 8, :].astype(F32)
                    s, m = s + v, jnp.maximum(m, v)
                gap = jnp.sum(s, axis=1, keepdims=True) * (1.0 / (H * W))
                gmp = jnp.max(m, axis=1, keepdims=True)
                w = w1f[c0:c0 + 8, :]
                ha = gap * w if ha is None else ha + gap * w
                hm = gmp * w if hm is None else hm + gmp * w
            ha = jnp.sum(ha, axis=0, keepdims=True)
            hm = jnp.sum(hm, axis=0, keepdims=True)
            hs = ha * (ha > 0).astype(F32) + hm * (hm > 0).astype(F32)

            done = {}

            def scale_of(c0):
                if c0 not in done:
                    z = jnp.sum(w2f[c0:c0 + 8, :] * hs, axis=1, keepdims=True)
                    sc = jax.nn.sigmoid(z).astype(BF16).astype(F32)
                    done[c0] = jnp.broadcast_to(sc, (8, LANES))
                    scale[c0:c0 + 8, :] = done[c0]
                return done[c0]

            for j in range(0, HEAD[0], 8):
                apply(j, [scale_of((p * SLAB + j) % C) for p in range(period)])
            start_write(0, HEAD[0])
            for c0 in range(0, C, 8):
                scale_of(c0)

            def wrap(c):
                return jnp.where(c >= C, c - C, c)

            def rows(j, c0):
                apply(j, [scale[pl.ds(pl.multiple_of(wrap(c0 + p * SLAB % C), 8), 8), :]
                          for p in range(period)])
                return wrap(c0 + 8)

            def piece(j0, n, c0):
                c0 = lax.fori_loop(0, n // 8, lambda g, c: rows(j0 + g * 8, c), c0)
                start_write(j0, n)
                return c0

            j0, c0 = HEAD[0], jnp.int32(HEAD[0] % C)
            for n in HEAD[1:]:
                c0 = piece(j0, n, c0)
                j0 += n
            c0 = lax.fori_loop(
                0, n_piece,
                lambda t, c: piece(pl.multiple_of(j0 + t * PIECE, 8), PIECE, c), c0)
            if tail:
                piece(SLAB - tail, tail, c0)

        pl.run_scoped(body, pltpu.SemaphoreType.DMA((n_read,)), pltpu.SemaphoreType.DMA(()))
        pltpu.make_async_copy(obuf, o_hbm, wsem).wait()

    return kernel


@jax.jit
def pallas_standalone__channel_attn_cbam__vision_kernel(
    x: jax.Array,
    w1: jax.Array,
    w2: jax.Array,
):
    B, H, W, C = x.shape
    hid = w1.shape[1]
    n_slab = H * C // SLAB
    xt = x.transpose(0, 1, 3, 2).reshape(H * C, W)
    out = pl.pallas_call(
        _make_kernel(H, C, W),
        in_specs=[pl.BlockSpec(memory_space=pltpu.HBM)] * 3,
        out_specs=pl.BlockSpec(memory_space=pltpu.HBM),
        out_shape=jax.ShapeDtypeStruct((n_slab, SLAB, W), x.dtype),
        scratch_shapes=[
            pltpu.VMEM((H * C, W), BF16),
            pltpu.VMEM((n_slab, SLAB, W), BF16),
            pltpu.VMEM((hid, C), BF16),
            pltpu.VMEM((hid, C), BF16),
            pltpu.VMEM((C, hid), F32),
            pltpu.VMEM((C, hid), F32),
            pltpu.VMEM((C, W), F32),
            pltpu.VMEM((C, W), F32),
            pltpu.VMEM((C, LANES), F32),
            pltpu.SemaphoreType.DMA(()),
        ],
        compiler_params=pltpu.CompilerParams(vmem_limit_bytes=64 * 2**20),
    )(xt, w1.T, w2)
    return out.reshape(B, H, C, W).transpose(0, 1, 3, 2)
```

```python
import math

import jax
import jax.numpy as jnp
from jax import lax
import jax.experimental.pallas as pl
import jax.experimental.pallas.tpu as pltpu

F32, BF16 = jnp.float32, jnp.bfloat16
LANES = 128

READ_CHUNKS = (124, 60, 24, 9, 4, 3)
SLAB = 2048
HEAD = (16, 16)
PIECE = 56


def _make_kernel(H, C, W, hid):
    n_slab = H * C // SLAB
    period = C // math.gcd(SLAB, C)
    n_piece = (SLAB - sum(HEAD)) // PIECE
    row0 = [sum(READ_CHUNKS[:i]) for i in range(len(READ_CHUNKS))]
    assert sum(READ_CHUNKS) == H and n_slab * SLAB == H * C and C % 16 == 0
    assert sum(HEAD) + n_piece * PIECE == SLAB
    assert LANES < W <= 2 * LANES and 2 * hid < LANES

    def kernel(x_hbm, w1t_hbm, w2_hbm, o_hbm, xbuf, obuf, w1v, w2v, w1f, w2f,
               acc_s, acc_m, scale, wsem):

        def body(rsem, psem):
            reads = [
                pltpu.make_async_copy(x_hbm.at[pl.ds(h0 * C, n * C)],
                                      xbuf.at[pl.ds(h0 * C, n * C)], rsem.at[i])
                for i, (h0, n) in enumerate(zip(row0, READ_CHUNKS))
            ]
            weights = [pltpu.make_async_copy(w1t_hbm, w1v, psem),
                       pltpu.make_async_copy(w2_hbm, w2v, psem)]

            def issue(i, carry):
                for k, copy in enumerate(weights + reads[1:]):
                    pl.when(i == k)(copy.start)
                return carry

            reads[0].start()
            lax.fori_loop(0, len(weights) + len(reads) - 1, issue, 0)

            acc_s[...] = jnp.zeros((C, W), F32)
            acc_m[...] = jnp.full((C, W), -jnp.inf, F32)
            for copy in weights:
                copy.wait()
            w1, w2 = w1v[...].astype(F32), w2v[...].astype(F32)
            pad = jnp.zeros((LANES - 2 * hid, C), F32)
            w1f[...] = jnp.concatenate([w1 * (1.0 / (H * W)), w1, pad], axis=0).T
            w2f[...] = jnp.concatenate([w2, w2, pad], axis=0).T

            for i in range(len(reads) - 1):
                n = READ_CHUNKS[i]
                u = max(d for d in range(1, 13) if n % d == 0)

                def channels(cg, carry, h0=row0[i], n=n, u=u):
                    c0 = pl.multiple_of(cg * 16, 16)

                    def step(b, sm):
                        s, m = sm
                        for q in range(u):
                            r = pl.multiple_of((h0 + b * u + q) * C + c0, 16)
                            v = xbuf[pl.ds(r, 16), :].astype(F32)
                            s, m = s + v, jnp.maximum(m, v)
                        return s, m

                    sm = (acc_s[pl.ds(c0, 16), :], acc_m[pl.ds(c0, 16), :])
                    s, m = step(0, sm) if n == u else lax.fori_loop(0, n // u, step, sm)
                    acc_s[pl.ds(c0, 16), :] = s
                    acc_m[pl.ds(c0, 16), :] = m
                    return carry

                reads[i].wait()
                lax.fori_loop(0, C // 16, channels, 0)

            reads[-1].wait()
            lane = lax.broadcasted_iota(jnp.int32, (8, LANES), 1)
            terms = []
            for c0 in range(0, C, 8):
                s, m = acc_s[c0:c0 + 8, :], acc_m[c0:c0 + 8, :]
                for h in range(row0[-1], H):
                    v = xbuf[h * C + c0:h * C + c0 + 8, :].astype(F32)
                    s, m = s + v, jnp.maximum(m, v)
                pooled = jnp.where(lane < hid, jnp.sum(s, axis=1, keepdims=True),
                                   jnp.max(m, axis=1, keepdims=True))
                terms.append(pooled * w1f[c0:c0 + 8, :])
            pre = sum(terms[2::2], terms[0]) + sum(terms[3::2], terms[1])
            pre = jnp.sum(pre, axis=0, keepdims=True)
            hidden = jnp.where(lane[:1] < 2 * hid, pre * (pre > 0).astype(F32), 0.0)

            gates = {}

            def gate(c0):
                if c0 not in gates:
                    z = jnp.sum(w2f[c0:c0 + 8, :] * hidden, axis=1, keepdims=True)
                    g = jax.nn.sigmoid(z).astype(BF16).astype(F32)
                    gates[c0] = jnp.broadcast_to(g, (8, LANES))
                    scale[c0:c0 + 8, :] = gates[c0]
                return gates[c0]

            def apply(j, gs):
                for p in range(period):
                    g = jnp.concatenate([gs[p], gs[p][:, :W - LANES]], axis=1)
                    for n in range(p, n_slab, period):
                        v = xbuf[pl.ds(pl.multiple_of(n * SLAB + j, 8), 8), :]
                        obuf[n, pl.ds(pl.multiple_of(j, 8), 8), :] = (
                            v.astype(F32) * g).astype(BF16)

            def start_write(j0, n):
                pltpu.make_async_copy(obuf.at[:, pl.ds(j0, n)],
                                      o_hbm.at[:, pl.ds(j0, n)], wsem).start()

            for j in range(0, HEAD[0], 8):
                apply(j, [gate((p * SLAB + j) % C) for p in range(period)])
            start_write(0, HEAD[0])
            for c0 in range(0, C, 8):
                gate(c0)

            def wrap(c):
                return jnp.where(c >= C, c - C, c)

            def piece(j0, n, c0):

                def rows(g, c):
                    apply(j0 + g * 8, [
                        scale[pl.ds(pl.multiple_of(wrap(c + p * SLAB % C), 8), 8), :]
                        for p in range(period)])
                    return wrap(c + 8)

                c0 = lax.fori_loop(0, n // 8, rows, c0)
                start_write(j0, n)
                return c0

            j0, c0 = HEAD[0], jnp.int32(HEAD[0] % C)
            for n in HEAD[1:]:
                c0 = piece(j0, n, c0)
                j0 += n
            lax.fori_loop(
                0, n_piece,
                lambda t, c: piece(pl.multiple_of(j0 + t * PIECE, 8), PIECE, c), c0)

        pl.run_scoped(body, pltpu.SemaphoreType.DMA((len(READ_CHUNKS),)),
                      pltpu.SemaphoreType.DMA(()))
        pltpu.make_async_copy(obuf, o_hbm, wsem).wait()

    return kernel


@jax.jit
def pallas_standalone__channel_attn_cbam__vision_kernel(
    x: jax.Array,
    w1: jax.Array,
    w2: jax.Array,
):
    B, H, W, C = x.shape
    hid = w1.shape[1]
    assert B == 1
    n_slab = H * C // SLAB
    xt = x.transpose(0, 1, 3, 2).reshape(H * C, W)
    out = pl.pallas_call(
        _make_kernel(H, C, W, hid),
        in_specs=[pl.BlockSpec(memory_space=pltpu.HBM)] * 3,
        out_specs=pl.BlockSpec(memory_space=pltpu.HBM),
        out_shape=jax.ShapeDtypeStruct((n_slab, SLAB, W), x.dtype),
        scratch_shapes=[
            pltpu.VMEM((H * C, W), BF16),
            pltpu.VMEM((n_slab, SLAB, W), BF16),
            pltpu.VMEM((hid, C), BF16),
            pltpu.VMEM((hid, C), BF16),
            pltpu.VMEM((C, LANES), F32),
            pltpu.VMEM((C, LANES), F32),
            pltpu.VMEM((C, W), F32),
            pltpu.VMEM((C, W), F32),
            pltpu.VMEM((C, LANES), F32),
            pltpu.SemaphoreType.DMA(()),
        ],
        compiler_params=pltpu.CompilerParams(vmem_limit_bytes=64 * 2**20),
    )(xt, w1.T, w2)
    return out.reshape(B, H, C, W).transpose(0, 1, 3, 2)
```
